```python
import os as _os
_os.environ.setdefault("JAX_PLATFORMS", "cpu")
import jax
import jax.numpy as jnp

def _softmax(x, axis=-1):
    return jax.nn.softmax(x, axis=axis)
def _gelu(x):
    return jax.nn.gelu(x, approximate=True)
def _silu(x):
    return jax.nn.silu(x)
def _sigmoid(x):
    return jax.nn.sigmoid(x)
def _layernorm(x, axis=-1, eps=1e-5):
    m = jnp.mean(x, axis=axis, keepdims=True)
    v = jnp.var(x, axis=axis, keepdims=True)
    return (x - m) / jnp.sqrt(v + eps)
def _scatter_add(tgt, idx, src, axis=0):
    return tgt.at[idx].add(src)
def _segment_sum(src, seg, n):
    return jax.ops.segment_sum(src, seg, n)
class _Rng:
    def __init__(self, key):
        self._k = key
    def _next(self):
        self._k, sub = jax.random.split(self._k)
        return sub
    def normal(self, shape):
        return jax.random.normal(self._next(), shape, dtype=jnp.bfloat16)
    def randint(self, lo, hi, shape):
        return jax.random.randint(self._next(), shape, lo, hi, dtype=jnp.int32)
    def uniform(self, shape, lo=0.0, hi=1.0):
        return jax.random.uniform(self._next(), shape, jnp.bfloat16, lo, hi)
    def permutation(self, n):
        return jax.random.permutation(self._next(), n)


kernel_name = 'sequential_preLN__softmax_full_mha__dense_activation_squared_relu__prompt'

def setup_inputs():
    _rng = _Rng(jax.random.key(int.from_bytes(__import__("os").urandom(4), "little")))
    _w = (lambda a: (lambda t: t.astype(jnp.bfloat16) if jnp.issubdtype(t.dtype, jnp.floating) else t)(jnp.asarray(a)))
    def _A_setup():
        B, S, D = 1, 2048, 640
        return {
            "x": _w((lambda *s: _rng.normal(s) * 0.05)(B, S, D)),
            "wqkv": _w((lambda *s: _rng.normal(s) * 0.05)(D, 3 * D)),
            "wo": _w((lambda *s: _rng.normal(s) * 0.05)(D, D)),
        }
    _A_in = _A_setup()

    def _B_setup():
        B, S, D, F = 1, 2048, 640, 1536
        return {
            "x": _w((lambda *s: _rng.normal(s) * 0.05)(B, S, D)),
            "w1": _w((lambda *s: _rng.normal(s) * 0.05)(D, F)),
            "b1": _w((lambda *s: _rng.normal(s) * 0.05)(F)),
            "w2": _w((lambda *s: _rng.normal(s) * 0.05)(F, D)),
            "b2": _w((lambda *s: _rng.normal(s) * 0.05)(D)),
        }
    _B_in = _B_setup()

    return {
        "A_x": _A_in["x"],
        "A_wqkv": _A_in["wqkv"],
        "A_wo": _A_in["wo"],
        "B_x": _B_in["x"],
        "B_w1": _B_in["w1"],
        "B_b1": _B_in["b1"],
        "B_w2": _B_in["w2"],
        "B_b2": _B_in["b2"],
    }

def reference(A_x, A_wqkv, A_wo, B_x, B_w1, B_b1, B_w2, B_b2):
    def _A_ref(x, wqkv, wo):
        B, S, D = x.shape
        H = 32; Dh = D // H
        qkv = (lambda x, *d: x.transpose(*d))((x @ wqkv).reshape(B, S, 3, H, Dh), 2, 0, 3, 1, 4)
        q, k, v = qkv[0], qkv[1], qkv[2]
        scale = Dh ** -0.5
        scores = jnp.einsum("bhqd,bhkd->bhqk", q, k) * scale
        p = _softmax(scores, axis=-1)
        o = jnp.einsum("bhqk,bhkd->bhqd", p, v)
        return (lambda x, *d: x.transpose(*d))(o, 0, 2, 1, 3).reshape(B, S, D) @ wo

    def _B_ref(x, w1, b1, w2, b2):
        h = jnp.einsum("bsd,df->bsf", x, w1) + b1
        zero = jnp.zeros_like(h)
        r = jnp.where(h > zero, h, zero)
        h = r * r
        out = jnp.einsum("bsf,fd->bsd", h, w2) + b2
        return out

    x = A_x
    h = x + _A_ref(_layernorm(x, axis=-1), A_wqkv, A_wo)
    h2 = h + _B_ref(_layernorm(h, axis=-1), B_w1, B_b1, B_w2, B_b2)
    return h2
```

```python
import functools
import math

import jax
import jax.numpy as jnp
from jax import lax
import jax.experimental.pallas as pl
import jax.experimental.pallas.tpu as pltpu

S, D, F, H = 2048, 640, 1536, 32
DH = D // H
BQ = 512
CK = 128
HG = 4
GR = HG * DH
NQ = S // BQ
NG = H // HG
EPS = 1e-5
F32, BF16 = jnp.float32, jnp.bfloat16


def _layernorm(x):
    m = jnp.mean(x, axis=-1, keepdims=True)
    xc = x - m
    v = jnp.mean(xc * xc, axis=-1, keepdims=True)
    return xc * lax.rsqrt(v + EPS)


def _kernel(x_hbm, wqkv_hbm, wo_hbm, w1_hbm, b1_ref, w2_hbm, b2_ref, out_hbm,
            x_v, wqkv_v, wo_v, w1_v, w2_v, k_s, qT_s, vT_s, oT_s, s_s, m_s, out_v,
            in_sem, out_sem):
    x_cp = [pltpu.make_async_copy(x_hbm.at[0, pl.ds(c * BQ, BQ), :], x_v.at[pl.ds(c * BQ, BQ), :], in_sem.at[c])
            for c in range(NQ)]
    w_cp = [pltpu.make_async_copy(src, dst, in_sem.at[NQ + i])
            for i, (src, dst) in enumerate(((wqkv_hbm, wqkv_v), (wo_hbm, wo_v), (w1_hbm, w1_v), (w2_hbm, w2_v)))]
    x_cp[0].start()
    w_cp[0].start()
    for c in x_cp[1:] + w_cp[1:]:
        c.start()

    qscale = DH ** -0.5 * math.log2(math.e)
    w_cp[0].wait()

    def qkv_chunk(c, carry):
        r0 = pl.multiple_of(c * BQ, BQ)
        pltpu.make_async_copy(x_hbm.at[0, pl.ds(r0, BQ), :], x_v.at[pl.ds(r0, BQ), :], in_sem.at[c]).wait()
        xn = _layernorm(x_v[pl.ds(r0, BQ), :].astype(F32)).astype(BF16)
        kk = jnp.dot(xn, wqkv_v[:, D:2 * D], preferred_element_type=F32).astype(BF16)
        for h in range(H):
            a = (h * DH) // 16 * 16
            k_s[h, pl.ds(r0, BQ), :] = kk[:, a:a + 32]
        q = jnp.dot(xn, wqkv_v[:, 0:D], preferred_element_type=F32) * qscale
        qT_s[c] = q.T.astype(BF16)
        v = jnp.dot(xn, wqkv_v[:, 2 * D:3 * D], preferred_element_type=F32).astype(BF16).astype(F32)
        vT_s[c] = v.T
        return carry

    lax.fori_loop(0, NQ, qkv_chunk, 0)

    row32 = lax.broadcasted_iota(jnp.int32, (32, BQ), 0)
    row24 = lax.broadcasted_iota(jnp.int32, (24, CK), 0)
    row8 = lax.broadcasted_iota(jnp.int32, (8, BQ), 0)
    nk = S // CK

    def q_weights(qb, g, i):
        r = pl.multiple_of(g * GR + 16 * i, 16)
        w = qT_s[qb, pl.ds(r, 32), :]
        keep = (row32 >= 4 * i) & (row32 < 4 * i + DH)
        return jnp.where(keep, w, jnp.zeros_like(w))

    def scores_step(w, h, slot, j):
        s = jnp.dot(k_s[h, j * CK:(j + 1) * CK, :], w, preferred_element_type=F32)
        s_s[slot, j * CK:(j + 1) * CK, :] = s
        return jnp.max(s.reshape(-1, 8, BQ), axis=0)

    def pv_step(g, i, slot, m, j):
        r = pl.multiple_of(g * GR + (0, 16, 40, 56)[i], 8)
        c, o = divmod(j * CK, BQ)
        vt = vT_s[c, pl.ds(r, 24), o:o + CK]
        ones = (row24 >= DH) if i % 2 == 0 else (row24 < 4)
        vt = jnp.where(ones, 1.0, vt)
        p = jnp.exp2(s_s[slot, j * CK:(j + 1) * CK, :] - m).astype(BF16)
        return jnp.dot(vt, p, preferred_element_type=F32)

    def normalise(acc, i):
        l = acc[DH:DH + 1] if i % 2 == 0 else acc[0:1]
        return acc * (1.0 / l)

    def store_heads(qb, g, o):
        r = pl.multiple_of(g * GR, 8)
        for pr in range(HG // 2):
            e, d = o[2 * pr], o[2 * pr + 1]
            mid = jnp.where(row8 < 4, e[16:24], d[0:8])
            oT_s[qb, pl.ds(r + 40 * pr, 40), :] = jnp.concatenate([e[0:16], mid, d[8:24]], axis=0)

    w = q_weights(0, 0, 0)
    m = None
    for j in range(nk):
        mm = scores_step(w, 0, 0, j)
        m = mm if m is None else jnp.maximum(m, mm)
    m_s[...] = jnp.max(m, axis=0, keepdims=True)

    def group(u, carry):
        qb, g = u // NG, u % NG
        un = jnp.minimum(u + 1, NQ * NG - 1)
        qbn, gn = un // NG, un % NG
        m_prev = m_s[...]
        outs = []
        for i in range(HG):
            if i + 1 < HG:
                w, hn = q_weights(qb, g, i + 1), g * HG + i + 1
            else:
                w, hn = q_weights(qbn, gn, 0), gn * HG
            m = acc = None
            for j in range(nk):
                mm = scores_step(w, hn, (i + 1) % 2, j)
                pv = pv_step(g, i, i % 2, m_prev, j)
                m = mm if m is None else jnp.maximum(m, mm)
                acc = pv if acc is None else acc + pv
            outs.append(normalise(acc, i))
            m_prev = jnp.max(m, axis=0, keepdims=True)
        m_s[...] = m_prev
        store_heads(qb, g, outs)
        return carry

    lax.fori_loop(0, NQ * NG, group, 0)

    for c in w_cp[1:]:
        c.wait()
    b1 = b1_ref[...].astype(F32).reshape(1, F)
    b2 = b2_ref[...].astype(F32).reshape(1, D)

    def out_copy(c):
        r0 = pl.multiple_of(c * BQ, BQ)
        return pltpu.make_async_copy(out_v.at[pl.ds(r0, BQ), :], out_hbm.at[0, pl.ds(r0, BQ), :], out_sem.at[c])

    def tail(c, carry):
        r0 = pl.multiple_of(c * BQ, BQ)
        o = oT_s[c].T.astype(BF16)
        h = x_v[pl.ds(r0, BQ), :].astype(F32) + jnp.dot(o, wo_v[...], preferred_element_type=F32)
        hn = _layernorm(h).astype(BF16)
        a = jnp.dot(hn, w1_v[...], preferred_element_type=F32) + b1
        a = jnp.maximum(a, 0.0)
        a = (a * a).astype(BF16)
        y = h + (jnp.dot(a, w2_v[...], preferred_element_type=F32) + b2)
        out_v[pl.ds(r0, BQ), :] = y.astype(BF16)
        out_copy(c).start()
        return carry

    lax.fori_loop(0, NQ, tail, 0)
    for c in range(NQ):
        out_copy(c).wait()


@jax.jit
def pallas_sequential_preLN__softmax_full_mha__dense_activation_squared_relu__prompt_kernel(
    A_x, A_wqkv, A_wo, B_x, B_w1, B_b1, B_w2, B_b2,
):
    del B_x
    hbm = pl.BlockSpec(memory_space=pl.ANY)
    vmem = pl.BlockSpec(memory_space=pltpu.VMEM)
    return pl.pallas_call(
        _kernel,
        out_shape=jax.ShapeDtypeStruct((1, S, D), BF16),
        in_specs=[hbm, hbm, hbm, hbm, vmem, hbm, vmem],
        out_specs=hbm,
        scratch_shapes=[
            pltpu.VMEM((S, D), BF16),
            pltpu.VMEM((D, 3 * D), BF16),
            pltpu.VMEM((D, D), BF16),
            pltpu.VMEM((D, F), BF16),
            pltpu.VMEM((F, D), BF16),
            pltpu.VMEM((H, S, 32), BF16),
            pltpu.VMEM((NQ, D, BQ), BF16),
            pltpu.VMEM((NQ, D, BQ), F32),
            pltpu.VMEM((NQ, D, BQ), F32),
            pltpu.VMEM((2, S, BQ), F32),
            pltpu.VMEM((1, BQ), F32),
            pltpu.VMEM((S, D), BF16),
            pltpu.SemaphoreType.DMA((NQ + 4,)),
            pltpu.SemaphoreType.DMA((NQ,)),
        ],
        compiler_params=pltpu.CompilerParams(vmem_limit_bytes=110 * 2**20),
    )(A_x, A_wqkv, A_wo, B_w1, B_b1, B_w2, B_b2)
```

```python
import math

import jax
import jax.numpy as jnp
from jax import lax
import jax.experimental.pallas as pl
import jax.experimental.pallas.tpu as pltpu

CFG = dict(G=(10, 10, 10, 10), K0=-0.659, SP=1.0, ST=2, TK=0, ORD="dg", GB=2, CP=14, LOOP=0, UNR=1, RB=64, QB=128, QW='v', LK=None, CG=1, AB=32, AO=128, N0=0, O3='iopx')

S, D, F, H = 2048, 640, 1536, 32
DH = D // H
VM = 24
BQ = 512
NT = BQ // 128
NB = S // BQ
CK = 128
G = CFG["G"]
GMAX = max(G)
ST = CFG["ST"]
LAG = NT
PM = 2 * NT
STEPS = NB * NB * NT
TB = 256
HB, KS, HF = TB // 2, 256, F // 2
EPS = 1e-5
Q_SCALE = DH ** -0.5 * math.log2(math.e)
L_MIN, L_MAX, V_MAX = 2.0 ** -60, 2.0 ** 100, 2.0 ** 20
F32, BF16, U32 = jnp.float32, jnp.bfloat16, jnp.uint32


def _layernorm(x):
    xc = x - jnp.mean(x, axis=-1, keepdims=True)
    return xc * lax.rsqrt(jnp.mean(xc * xc, axis=-1, keepdims=True) + EPS)


def _mm(a, b):
    return jnp.dot(a, b, preferred_element_type=F32)


def _tile(t):
    return slice(t * 128, (t + 1) * 128)


def _ds(start, size, align):
    return pl.ds(start if isinstance(start, int) else pl.multiple_of(start, align), size)


def _pack(a, b):
    return jnp.concatenate(
        [pltpu.bitcast(jnp.concatenate([a[:, _tile(t)], b[:, _tile(t)]], axis=0).astype(BF16), U32)
         for t in range(a.shape[1] // 128)], axis=1)


def _lhs_terms(a11, a12, a21, a22):
    return a11 + a22, a21 + a22, a11, a22, a11 + a12, a21 - a11, a12 - a22


def _rhs_terms(b11, b12, b21, b22):
    return b11 + b22, b11, b12 - b22, b21 - b11, b22, b11 + b12, b21 + b22


def _quadrants(m1, m2, m3, m4, m5, m6, m7):
    return m1 + m4 - m5 + m7, m3 + m5, m2 + m4, m1 - m2 + m3 + m6


def _split(a, r, c):
    return a[:r, :c], a[:r, c:2 * c], a[r:2 * r, :c], a[r:2 * r, c:2 * c]


def _join(c11, c12, c21, c22):
    return jnp.concatenate([jnp.concatenate([c11, c12], axis=1), jnp.concatenate([c21, c22], axis=1)], axis=0)


def _step(t):
    return t // (NB * NT), t // NT % NB, t % NT


def _kernel(x_hbm, wqkv_hbm, wo_hbm, w1_hbm, b1_hbm, w2_hbm, b2_hbm, out_hbm,
            x_v, wq_v, wk_v, wv_v, wo_v, w1_v, w2_v, b1_v, b2_v,
            xn_s, kraw_s, k_s, kf_s, qw_s, qf_s, vt_s, o_s, kb0, kb1, ok_s, out_v,
            h_s, hn_s, hr_s, a_s, w1_s, w2_s, in_sem, out_sem, *pm):
    def x_copy(c):
        r = _ds(c * BQ, BQ, BQ)
        return pltpu.make_async_copy(x_hbm.at[0, r, :], x_v.at[r, :], in_sem.at[c])

    x_cp = [x_copy(c) for c in range(NB)]
    wk_cp, wo_cp, *w_cp = [pltpu.make_async_copy(src, dst, in_sem.at[NB + i]) for i, (src, dst) in enumerate((
        (wqkv_hbm.at[:, pl.ds(D, D)], wk_v), (wo_hbm, wo_v),
        (wqkv_hbm.at[:, pl.ds(2 * D, D)], wv_v), (wqkv_hbm.at[:, pl.ds(0, D)], wq_v),
        (w1_hbm, w1_v), (w2_hbm, w2_v), (b1_hbm, b1_v.at[0]), (b2_hbm, b2_v.at[0])))]

    with jax.named_scope("ph0"):
        for cp in [x_cp[0], wk_cp] + x_cp[1:] + w_cp[:3]:
            cp.start()
        ok_s[0] = jnp.ones((8, BQ), F32)
        for buf in pm:
            buf[...] = jnp.zeros(buf.shape, U32)
        o_s[0, NB - 1] = jnp.zeros((VM, BQ), F32)
        wk_cp.wait()

    def window(h):
        return h * DH // 16 * 16

    def project_keys(half, carry):
        RB = CFG["RB"]

        def normed(r):
            c, o = 2 * half + r // BQ, r % BQ
            xn = _layernorm(x_v[_ds(c * BQ + o, RB, RB), :].astype(F32)).astype(BF16)
            xn_s[c, o:o + RB, :] = xn
            return xn

        x_copy(2 * half).wait()
        xn = normed(0)
        for r0 in range(0, 2 * BQ, RB):
            if r0 + RB == BQ:
                x_copy(2 * half + 1).wait()
            k = _mm(xn, wk_v[...])
            if r0 + RB < 2 * BQ:
                xn = normed(r0 + RB)
            c, o = 2 * half + r0 // BQ, r0 % BQ
            for r in range(0, RB, 16):
                kraw_s[c, (o + r) // 2:(o + r) // 2 + 8, :] = _pack(k[r:r + 8], k[r + 8:r + 16])
        return carry

    def store_keys(c):
        k = kraw_s[c]
        k_vpu = pltpu.bitcast(k[(BQ - 8 * GMAX) // 2:], BF16).astype(F32)
        for h in range(H):
            t, off = divmod(window(h), 128)
            win = k[:, _tile(t)]
            if off:
                win = pltpu.roll(win, 128 - off, axis=1)
            if off + 32 > 128:
                lane = lax.broadcasted_iota(jnp.int32, win.shape, 1)
                win = jnp.where(lane < 128 - off, win, pltpu.roll(k[:, _tile(t + 1)], 128 - off, axis=1))
            k_s[h, c] = win
            kf_s[h, c] = k_vpu[:, h * DH:(h + 1) * DH]

    def store_queries(c, q):
        q = (q * Q_SCALE).astype(BF16).astype(F32).T
        row = lax.broadcasted_iota(jnp.int32, (8, BQ), 0)
        for h in range(H):
            w = []
            for r in range(window(h), window(h) + 32, 8):
                lo, hi = h * DH - r, (h + 1) * DH - r
                if lo >= 8 or hi <= 0:
                    w.append(jnp.zeros((8, BQ), F32))
                elif lo > 0 or hi < 8:
                    w.append(jnp.where((row >= lo) & (row < hi), q[r:r + 8], 0.0))
                else:
                    w.append(q[r:r + 8])
            qw_s[h, c, 0:8, :] = _pack(w[0], w[1])
            qw_s[h, c, 8:16, :] = _pack(w[2], w[3])
            qf_s[h, c, 0:DH, :] = q[h * DH:(h + 1) * DH]

    def store_values(c, v):
        v = v.astype(BF16).astype(F32).T
        small = jnp.where(jnp.abs(v) <= V_MAX, 1.0, 0.0)
        ok_s[0] = jnp.minimum(ok_s[0], jnp.min(small.reshape(D // 8, 8, BQ), axis=0))
        for h in range(H):
            vt_s[h, c, 0:DH, :] = v[h * DH:(h + 1) * DH]
            vt_s[h, c, DH:VM, :] = jnp.ones((VM - DH, BQ), F32)

    def spread_keys(kb, k, groups, items):
        for i in items:
            d, g = divmod(i, groups) if CFG["ORD"] == "dg" else divmod(i, DH)[::-1]
            r = 8 * (GMAX - groups + g)
            kb[(g * DH + d) * 8:(g * DH + d + 1) * 8, :] = jnp.broadcast_to(k(slice(r, r + 8), slice(d, d + 1)), (8, 128))

    def strassen_weights(ref, w_v, rows, cols, r):
        top = w_v[_ds(r, 16, 16), 0:2 * cols].astype(F32)
        bot = w_v[_ds(rows + r, 16, 16), 0:2 * cols].astype(F32)
        token = None
        for i, term in enumerate(_rhs_terms(top[:, :cols], top[:, cols:], bot[:, :cols], bot[:, cols:])):
            packed = _pack(term[0:8], term[8:16])
            ref[i, _ds(r // 2, 8, 8), :] = packed
            for t in range(cols // 128):
                token = packed[:, _tile(t)] if token is None else token | packed[:, _tile(t)]
        return token

    def beside(lhs, zero, jobs):
        token = None
        for job in jobs:
            t = strassen_weights(*job)
            token = t if token is None else token | t
        always = lax.broadcasted_iota(jnp.int32, (16, 128), 0) >= zero
        corner = jnp.where(always, lhs[0:16, 0:128], pltpu.bitcast(token, BF16))
        return jnp.concatenate([jnp.concatenate([corner, lhs[0:16, 128:]], axis=1), lhs[16:]], axis=0)

    def project_queries_values(half, carry):
        jobs = [(w1_s, w1_v, KS, HF, half * (KS // 2) + r) for r in range(0, KS // 2, 16)] if CFG["QB"] else []

        def project(c, w_v, busy):
            if not (jobs and busy):
                return _mm(xn_s[c], w_v[...])
            return jnp.concatenate(
                [_mm(beside(xn_s[c, r:r + CFG["QB"], :], lax.shift_right_logical(half, 10), [jobs.pop()]), w_v[...])
                 for r in range(0, BQ, CFG["QB"])], axis=0)

        for i in range(2):
            c = 2 * half + i
            q = project(c, wq_v, 'q' in CFG['QW'])
            store_keys(c)
            if i == 0:
                k0 = pltpu.bitcast(kraw_s[0, (BQ - 8 * GMAX) // 2:, 0:128], BF16).astype(F32)
                spread_keys(kb0, lambda r, d: k0[r, d], G[0], range(G[0] * DH))
            v = project(c, wv_v, 'v' in CFG['QW'])
            store_queries(c, q)
            store_values(c, v)
        assert not jobs
        return carry

    with jax.named_scope("ph1"):
        if CFG["LOOP"]:
            for cp in x_cp + w_cp[:3]:
                cp.wait()
        else:
            lax.fori_loop(0, 2, project_keys, 0)
            for cp in w_cp[:3]:
                cp.wait()
            lax.fori_loop(0, 2, project_queries_values, 0)
        for cp in [wo_cp] + w_cp[3:]:
            cp.start()

    def query_weights(h, qb):
        return jnp.concatenate([pltpu.bitcast(qw_s[h, qb], BF16), jnp.zeros((96, BQ), BF16)], axis=0)

    def accumulate(t0, h, slot, zero, acc):
        parts = []
        for t in range(t0, t0 + ST):
            kblk, qb, u = _step(t)
            p = pltpu.bitcast(pm[t % PM][_ds(zero * 8, CK // 2, 8), :], BF16)
            parts.append(_mm(vt_s[h, kblk, :, _tile(u)], p))
            acc = parts[-1] if u == 0 else acc + parts[-1]
            if u == NT - 1:
                o_s[slot, qb] = acc + o_s[slot, qb] if kblk else acc
        return acc, parts

    def check(slot, qb, ok, counts=True, pace=lambda l: l):
        l = pace(jnp.broadcast_to(o_s[slot, qb, DH:DH + 1, :], (8, BQ)))
        return jnp.where(((l >= L_MIN) & (l <= L_MAX)) | jnp.logical_not(counts), ok, 0.0)

    def head(h, carry):
        zero = lax.shift_right_logical(h, 10)
        always = lax.broadcasted_iota(jnp.int32, (8, 128), 0) >= zero
        history, acc, ok = [], None, ok_s[0]
        for t0 in range(0, STEPS, ST):
            kblk, qb, u0 = _step(t0)
            groups, mxu_keys = G[kblk], BQ - 8 * G[kblk]

            def put(r, lanes, a, b):
                pm[(t0 - u0 + r // CK) % PM][r % CK // 2:r % CK // 2 + 8, lanes] = _pack(a, b)

            lo, hi = (mxu_keys * u // NT // 16 * 16 if u < NT else mxu_keys for u in (u0, u0 + ST))
            s = _mm(pltpu.bitcast(k_s[h, kblk, lo // 2:hi // 2, :], BF16), query_weights(h, qb))
            e = jnp.exp2(s)
            for r in range(0, hi - lo, 16):
                for t in range(NT):
                    put(lo + r, _tile(t), e[r:r + 8, _tile(t)], e[r + 8:r + 16, _tile(t)])
            if t0 >= LAG:
                acc, parts = accumulate(t0 - LAG, h, h + 1, zero, acc)
            else:
                acc, parts = accumulate(STEPS - LAG + t0, jnp.maximum(h - 1, 0), h, zero, acc)

            tk = _tile(CFG["TK"])
            history.append([s[r:r + 8, tk] for r in range(0, hi - lo, 8)]
                           + [part[r:r + 8, tk] for part in parts for r in range(0, VM, 8)])
            kb, kb_next = (kb0, kb1) if kblk % 2 == 0 else (kb1, kb0)
            for u in range(u0, u0 + ST):
                q = [jnp.broadcast_to(qf_s[h, qb, d:d + 1, _tile(u)], (8, 128)) for d in range(DH)]
                for d in range(DH):
                    when = (u - u0 + CFG["K0"] + CFG["SP"] * d / DH) / ST
                    if CFG["LK"] is not None and t0 + ST == STEPS:
                        when = min(when, CFG["LK"] * (1 + when) - 1) if when > 0 else when
                    back = -math.floor(when)
                    if back < len(history):
                        results = history[-1 - back]
                        q[d] = jnp.where(always, q[d], results[int(len(results) * (when + back))])
                scores = [None] * groups
                gb = CFG["GB"] or groups
                for g0 in range(0, groups, gb):
                    for d in range(DH):
                        for g in range(g0, min(g0 + gb, groups)):
                            term = kb[(g * DH + d) * 8:(g * DH + d + 1) * 8, :] * q[d]
                            scores[g] = term if d == 0 else scores[g] + term
                for g in range(0, groups, 2):
                    put(mxu_keys + 8 * g, _tile(u), jnp.exp2(scores[g]), jnp.exp2(scores[g + 1]))
                i, n, nxt = qb * NT + u, NB * NT, (kblk + 1) % NB
                h_nxt = h if nxt else jnp.minimum(h + 1, H - 1)
                spread_keys(kb_next, lambda r, d: kf_s[h_nxt, nxt, r, d], G[nxt],
                            range(G[nxt] * DH * i // n, G[nxt] * DH * (i + 1) // n))
                if i == CFG["CP"]:
                    wide = jnp.concatenate([always] * NT, axis=1)
                    pace = (lambda l: jnp.where(wide, l, s[0:8])) if CFG["CG"] else (lambda l: l)
                    ok = check(h, kblk, ok, h > 0, pace)
        ok_s[0] = ok
        return carry + zero

    with jax.named_scope("ph2"):
        zero = lax.fori_loop(0, H, head, 0, unroll=CFG["UNR"])
        acc, ok = None, ok_s[0]
        for t0 in range(STEPS - LAG, STEPS, ST):
            acc, _ = accumulate(t0, H - 1, H, 0, acc)
        for qb in range(NB):
            ok = check(H, qb, ok)

    @pl.when(jnp.min(ok) < 0.5)
    def _():
        def shifted_softmax(i, carry):
            h, qb = i // NB, i % NB
            w = query_weights(h, qb)

            def scores(c):
                return _mm(pltpu.bitcast(k_s[h, c], BF16), w)

            m = lax.fori_loop(0, NB, lambda c, m: jnp.maximum(m, jnp.max(scores(c), axis=0, keepdims=True)),
                              jnp.full((1, BQ), -jnp.inf, F32))
            o_s[h + 1, qb] = lax.fori_loop(
                0, NB, lambda c, o: o + _mm(vt_s[h, c], jnp.exp2(scores(c) - m).astype(BF16)), jnp.zeros((VM, BQ), F32))
            return carry

        lax.fori_loop(0, H * NB, shifted_softmax, 0)

    with jax.named_scope("ph3"):
        wo_cp.wait()
        for cp in w_cp[3:]:
            cp.wait()
        if CFG["LOOP"]:
            return
        b1, b2 = (jnp.concatenate([b[i:i + 1] for i in range(b.shape[0])], axis=1)
                  for b in (b1_v[0].astype(F32), b2_v[0].astype(F32)))

        def rows(j):
            return _ds(j * TB, TB, TB)

        def attend(j, jobs=()):
            def head_rows(h):
                acc = o_s[h + 1, j // 2, :, _ds(j % 2 * TB, TB, TB)]
                inv = 1.0 / jnp.broadcast_to(acc[DH:DH + 1], (8, TB))
                return jnp.concatenate([acc[r:r + 8] * inv for r in range(0, VM, 8)], axis=0)[0:DH]

            att = jnp.concatenate([head_rows(h) for h in range(H)], axis=0).T
            ab = CFG["AB"] if jobs else CFG["AO"]
            parts = [att[r:r + ab].astype(BF16) for r in range(0, TB, ab)]
            if jobs:
                parts = [beside(part, zero, jobs[i::len(parts)]) for i, part in enumerate(parts)]
            res = x_v[rows(j), :].astype(F32) + jnp.concatenate([_mm(part, wo_v[...]) for part in parts], axis=0)
            h_s[j % 4] = res
            hn = _layernorm(res)
            for i, term in enumerate(_lhs_terms(*_split(hn, HB, KS))):
                hn_s[i] = term.astype(BF16)
            hr_s[...] = hn[:, 2 * KS:].astype(BF16)

        def hidden_inputs():
            return [hn_s[i] for i in range(7)], hr_s[...]

        def hidden(terms, rest, jobs=()):
            if jobs:
                terms = [beside(term, zero, jobs[i::7]) for i, term in enumerate(terms)]
            extra = _split(_mm(rest, w1_v[2 * KS:, :]) + b1, HB, HF)
            quads = _quadrants(*[_mm(term, pltpu.bitcast(w1_s[i], BF16)) for i, term in enumerate(terms)])
            return [jnp.square(jnp.maximum(q + e, 0.0)) for q, e in zip(quads, extra)]

        def store_hidden(a):
            for i, term in enumerate(_lhs_terms(*a) + (a[1], a[2])):
                a_s[i] = term.astype(BF16)

        def output_wide(j):
            y = _join(*_quadrants(*[_mm(a_s[i], pltpu.bitcast(w2_s[i], BF16)) for i in range(7)]))
            out_v[rows(j), 0:2 * KS] = (h_s[j % 4, :, 0:2 * KS] + (y + b2[:, 0:2 * KS])).astype(BF16)
            return _join(a_s[2], a_s[7], a_s[8], a_s[3])

        def output_rest(j, a):
            y = _mm(a, w2_v[:, 2 * KS:]) + b2[:, 2 * KS:]
            out_v[rows(j), 2 * KS:] = (h_s[j % 4, :, 2 * KS:] + y).astype(BF16)

        def out_copy(i, r):
            return pltpu.make_async_copy(out_v.at[r, :], out_hbm.at[0, r, :], out_sem.at[i])

        def feed_forward(j, carry):
            inputs = hidden_inputs()
            a = output_wide(j)
            attend(j + 2)
            store_hidden(hidden(*inputs))
            output_rest(j, a)
            out_copy(j, rows(j)).start()
            return carry

        n = S // TB
        jobs = [] if CFG['QB'] else [(w1_s, w1_v, KS, HF, r) for r in range(0, KS, 16)]
        n0 = CFG["N0"]
        attend(0, jobs[:n0])
        inputs = hidden_inputs()
        attend(1, jobs[n0:])
        store_hidden(hidden(*inputs, [(w2_s, w2_v, HF, KS, r) for r in range(0, HF, 16)]))
        lax.fori_loop(0, n - 2, feed_forward, 0)
        a_last = hidden(*hidden_inputs())
        output_rest(n - 2, output_wide(n - 2))
        out_copy(n - 2, rows(n - 2)).start()
        halves = [pl.ds(S - TB + r, HB) for r in (0, HB)]
        for i, r in enumerate(halves):
            a = jnp.concatenate(a_last[2 * i:2 * i + 2], axis=1).astype(BF16)
            out_v[r, :] = (h_s[(n - 1) % 4, i * HB:(i + 1) * HB, :] + (_mm(a, w2_v[...]) + b2)).astype(BF16)
            out_copy(n - 1 + i, r).start()
    with jax.named_scope("ph4"):
        for i, r in enumerate([rows(j) for j in range(n - 1)] + halves):
            out_copy(i, r).wait()


@jax.jit
def pallas_sequential_preLN__softmax_full_mha__dense_activation_squared_relu__prompt_kernel(
    A_x: jax.Array,
    A_wqkv: jax.Array,
    A_wo: jax.Array,
    B_x: jax.Array,
    B_w1: jax.Array,
    B_b1: jax.Array,
    B_w2: jax.Array,
    B_b2: jax.Array,
):
    del B_x
    hbm = pl.BlockSpec(memory_space=pl.ANY)
    scratch = [
        pltpu.VMEM((S, D), BF16),
        pltpu.VMEM((D, D), BF16),
        pltpu.VMEM((D, D), BF16),
        pltpu.VMEM((D, D), BF16),
        pltpu.VMEM((D, D), BF16),
        pltpu.VMEM((D, F), BF16),
        pltpu.VMEM((F, D), BF16),
        pltpu.VMEM((7, F // 128, 128), BF16),
        pltpu.VMEM((2, D // 128, 128), BF16),
        pltpu.VMEM((NB, BQ, D), BF16),
        pltpu.VMEM((NB, BQ // 2, D), U32),
        pltpu.VMEM((H, NB, BQ // 2, 128), U32),
        pltpu.VMEM((H, NB, 8 * GMAX, DH), F32),
        pltpu.VMEM((H, NB, 16, BQ), U32),
        pltpu.VMEM((H, NB, VM, BQ), F32),
        pltpu.VMEM((H, NB, VM, BQ), F32),
        pltpu.VMEM((H + 1, NB, VM, BQ), F32),
        pltpu.VMEM((GMAX * DH * 8, 128), F32),
        pltpu.VMEM((GMAX * DH * 8, 128), F32),
        pltpu.VMEM((2, 8, BQ), F32),
        pltpu.VMEM((S, D), BF16),
        pltpu.VMEM((4, TB, D), F32),
        pltpu.VMEM((7, HB, KS), BF16),
        pltpu.VMEM((TB, D - 2 * KS), BF16),
        pltpu.VMEM((9, HB, HF), BF16),
        pltpu.VMEM((7, KS // 2, HF), U32),
        pltpu.VMEM((7, HF // 2, KS), U32),
        pltpu.SemaphoreType.DMA((NB + 8,)),
        pltpu.SemaphoreType.DMA((S // TB + 1,)),
    ]
    scratch += [pltpu.VMEM((CK // 2, BQ), U32)] * PM
    return pl.pallas_call(
        _kernel,
        out_shape=jax.ShapeDtypeStruct((1, S, D), BF16),
        in_specs=[hbm] * 7,
        out_specs=hbm,
        scratch_shapes=scratch,
        compiler_params=pltpu.CompilerParams(vmem_limit_bytes=100 * 2**20),
    )(A_x, A_wqkv, A_wo, B_w1, B_b1.reshape(F // 128, 128), B_w2, B_b2.reshape(D // 128, 128))
```

```python
import math

import jax
import jax.numpy as jnp
from jax import lax
import jax.experimental.pallas as pl
import jax.experimental.pallas.tpu as pltpu

S, D, F, H = 2048, 640, 1536, 32
DH = D // H
VM = 24
BQ = 512
NT = BQ // 128
NB = S // BQ
CK = 128
G = 10
MXU_KEYS = BQ - 8 * G
ST = 2
LAG = NT
PM = 2 * NT
STEPS = NB * NB * NT
TB = 256
HB, KS, HF = TB // 2, 256, F // 2
RB = 64
X0 = 320
EPS = 1e-5
Q_SCALE = DH ** -0.5 * math.log2(math.e)
L_MIN, L_MAX, V_MAX = 2.0 ** -60, 2.0 ** 100, 2.0 ** 20
F32, BF16, U32 = jnp.float32, jnp.bfloat16, jnp.uint32


def _layernorm(x):
    xc = x - jnp.mean(x, axis=-1, keepdims=True)
    return xc * lax.rsqrt(jnp.mean(xc * xc, axis=-1, keepdims=True) + EPS)


def _mm(a, b):
    return jnp.dot(a, b, preferred_element_type=F32)


def _tile(t):
    return slice(t * 128, (t + 1) * 128)


def _ds(start, size, align):
    return pl.ds(start if isinstance(start, int) else pl.multiple_of(start, align), size)


def _pack(a, b):
    return jnp.concatenate(
        [pltpu.bitcast(jnp.concatenate([a[:, _tile(t)], b[:, _tile(t)]], axis=0).astype(BF16), U32)
         for t in range(a.shape[1] // 128)], axis=1)


def _lhs_terms(a11, a12, a21, a22):
    return a11 + a22, a21 + a22, a11, a22, a11 + a12, a21 - a11, a12 - a22


def _rhs_terms(b11, b12, b21, b22):
    return b11 + b22, b11, b12 - b22, b21 - b11, b22, b11 + b12, b21 + b22


def _quadrants(m1, m2, m3, m4, m5, m6, m7):
    return m1 + m4 - m5 + m7, m3 + m5, m2 + m4, m1 - m2 + m3 + m6


def _products(order, lhs, rhs):
    m = {i: _mm(lhs(i), rhs(i)) for i in order}
    return [m[i] for i in range(7)]


def _split(a, r, c):
    return a[:r, :c], a[:r, c:2 * c], a[r:2 * r, :c], a[r:2 * r, c:2 * c]


def _join(c11, c12, c21, c22):
    return jnp.concatenate([jnp.concatenate([c11, c12], axis=1), jnp.concatenate([c21, c22], axis=1)], axis=0)


def _step(t):
    return t // (NB * NT), t // NT % NB, t % NT


def _kernel(x_hbm, wqkv_hbm, wo_hbm, w1_hbm, b1_hbm, w2_hbm, b2_hbm, out_hbm,
            x_v, wq_v, wk_v, wv_v, wo_v, w1_v, w2_v, b1_v, b2_v,
            xn_s, kraw_s, k_s, kf_s, qw_s, qf_s, vt_s, o_s, kb0, kb1, ok_s, out_v,
            h_s, hn_s, hr_s, a_s, w1_s, w2_s, in_sem, out_sem, *pm):
    def x_copy(half, part):
        r = _ds(half * (S // 2) + part * X0, S // 2 - X0 if part else X0, RB)
        return pltpu.make_async_copy(x_hbm.at[0, r, :], x_v.at[r, :], in_sem.at[2 * half + part])

    x_cp = [x_copy(half, part) for half in range(2) for part in range(2)]
    wk_cp, wo_cp, *w_cp = [pltpu.make_async_copy(src, dst, in_sem.at[NB + i]) for i, (src, dst) in enumerate((
        (wqkv_hbm.at[:, pl.ds(D, D)], wk_v), (wo_hbm, wo_v),
        (wqkv_hbm.at[:, pl.ds(2 * D, D)], wv_v), (wqkv_hbm.at[:, pl.ds(0, D)], wq_v),
        (w1_hbm, w1_v), (w2_hbm, w2_v), (b1_hbm, b1_v.at[0]), (b2_hbm, b2_v.at[0])))]

    for cp in [x_cp[0], wk_cp] + x_cp[1:] + w_cp[:3]:
        cp.start()
    ok_s[0] = jnp.ones((8, BQ), F32)
    for t in range(STEPS - LAG, STEPS):
        pm[t % PM][...] = jnp.zeros((CK // 2, BQ), U32)
    o_s[0] = jnp.ones((NB, VM, BQ), F32)
    x_cp[0].wait()
    xn_s[0, 0:RB, :] = _layernorm(x_v[0:RB, :].astype(F32)).astype(BF16)
    wk_cp.wait()

    def window(h):
        return h * DH // 16 * 16

    def project_keys(half, carry):
        def normed(r):
            c, o = 2 * half + r // BQ, r % BQ
            xn = _layernorm(x_v[_ds(c * BQ + o, RB, RB), :].astype(F32)).astype(BF16)
            xn_s[c, o:o + RB, :] = xn
            return xn

        @pl.when(half == 1)
        def _():
            x_cp[2].wait()
            normed(0)

        xn = xn_s[2 * half, 0:RB, :]
        for r0 in range(0, 2 * BQ, RB):
            if r0 + RB == X0:
                x_copy(half, 1).wait()
            k = _mm(xn, wk_v[...])
            if r0 + RB < 2 * BQ:
                xn = normed(r0 + RB)
            c, o = 2 * half + r0 // BQ, r0 % BQ
            for r in range(0, RB, 16):
                kraw_s[c, (o + r) // 2:(o + r) // 2 + 8, :] = _pack(k[r:r + 8], k[r + 8:r + 16])
        return carry

    def store_keys(c):
        k = kraw_s[c]
        k_vpu = pltpu.bitcast(k[MXU_KEYS // 2:], BF16).astype(F32)
        for h in range(H):
            t, off = divmod(window(h), 128)
            win = k[:, _tile(t)]
            if off:
                win = pltpu.roll(win, 128 - off, axis=1)
            if off + 32 > 128:
                lane = lax.broadcasted_iota(jnp.int32, win.shape, 1)
                win = jnp.where(lane < 128 - off, win, pltpu.roll(k[:, _tile(t + 1)], 128 - off, axis=1))
            k_s[h, c] = win
            kf_s[h, c] = k_vpu[:, h * DH:(h + 1) * DH]

    def store_queries(c, q):
        q = (q * Q_SCALE).astype(BF16).astype(F32).T
        row = lax.broadcasted_iota(jnp.int32, (8, BQ), 0)
        for h in range(H):
            w = []
            for r in range(window(h), window(h) + 32, 8):
                lo, hi = h * DH - r, (h + 1) * DH - r
                if lo >= 8 or hi <= 0:
                    w.append(jnp.zeros((8, BQ), F32))
                elif lo > 0 or hi < 8:
                    w.append(jnp.where((row >= lo) & (row < hi), q[r:r + 8], 0.0))
                else:
                    w.append(q[r:r + 8])
            qw_s[h, c, 0:8, :] = _pack(w[0], w[1])
            qw_s[h, c, 8:16, :] = _pack(w[2], w[3])
            qf_s[h, c, 0:DH, :] = q[h * DH:(h + 1) * DH]

    def store_values(c, v):
        v = v.astype(BF16).astype(F32).T
        small = jnp.where(jnp.abs(v) <= V_MAX, 1.0, 0.0)
        ok_s[0] = jnp.minimum(ok_s[0], jnp.min(small.reshape(D // 8, 8, BQ), axis=0))
        for h in range(H):
            vt_s[h, c, 0:DH, :] = v[h * DH:(h + 1) * DH]
            vt_s[h, c, DH:VM, :] = jnp.ones((VM - DH, BQ), F32)

    def spread_keys(kb, k, items):
        for i in items:
            d, g = divmod(i, G)
            kb[(g * DH + d) * 8:(g * DH + d + 1) * 8, :] = jnp.broadcast_to(k(slice(8 * g, 8 * g + 8), slice(d, d + 1)), (8, 128))

    def strassen_weights(ref, w_v, rows, cols, r):
        top = w_v[_ds(r, 16, 16), 0:2 * cols].astype(F32)
        bot = w_v[_ds(rows + r, 16, 16), 0:2 * cols].astype(F32)
        token = None
        for i, term in enumerate(_rhs_terms(top[:, :cols], top[:, cols:], bot[:, :cols], bot[:, cols:])):
            packed = _pack(term[0:8], term[8:16])
            ref[i, _ds(r // 2, 8, 8), :] = packed
            for t in range(cols // 128):
                token = packed[:, _tile(t)] if token is None else token | packed[:, _tile(t)]
        return token

    def beside(lhs, zero, jobs):
        token = None
        for job in jobs:
            t = strassen_weights(*job)
            token = t if token is None else token | t
        always = lax.broadcasted_iota(jnp.int32, (16, 128), 0) >= zero
        corner = jnp.where(always, lhs[0:16, 0:128], pltpu.bitcast(token, BF16))
        return jnp.concatenate([jnp.concatenate([corner, lhs[0:16, 128:]], axis=1), lhs[16:]], axis=0)

    def project_queries_values(half, carry):
        zero = lax.shift_right_logical(half, 10)
        jobs = [(w1_s, w1_v, KS, HF, half * (KS // 2) + r) for r in range(0, KS // 2, 16)]
        for i in range(2):
            c = 2 * half + i
            q = _mm(xn_s[c], wq_v[...])
            store_keys(c)
            if i == 0:
                k0 = pltpu.bitcast(kraw_s[0, MXU_KEYS // 2:, 0:128], BF16).astype(F32)
                spread_keys(kb0, lambda r, d: k0[r, d], range(G * DH))
            v = jnp.concatenate([_mm(beside(xn_s[c, r:r + 128, :], zero, [jobs.pop()]), wv_v[...])
                                 for r in range(0, BQ, 128)], axis=0)
            store_queries(c, q)
            store_values(c, v)
        return carry

    lax.fori_loop(0, 2, project_keys, 0)
    for cp in w_cp[:3]:
        cp.wait()
    lax.fori_loop(0, 2, project_queries_values, 0)
    for cp in [wo_cp] + w_cp[3:]:
        cp.start()

    def query_weights(h, qb):
        return jnp.concatenate([pltpu.bitcast(qw_s[h, qb], BF16), jnp.zeros((96, BQ), BF16)], axis=0)

    def accumulate(t0, h, slot, zero, acc):
        parts = []
        for t in range(t0, t0 + ST):
            kblk, qb, u = _step(t)
            p = pltpu.bitcast(pm[t % PM][_ds(zero * 8, CK // 2, 8), :], BF16)
            parts.append(_mm(vt_s[h, kblk, :, _tile(u)], p))
            acc = parts[-1] if u == 0 else acc + parts[-1]
            if u == NT - 1:
                o_s[slot, qb] = acc + o_s[slot, qb] if kblk else acc
        return acc, parts

    def check(slot, qb, ok):
        l = jnp.broadcast_to(o_s[slot, qb, DH:DH + 1, :], (8, BQ))
        return jnp.where((l >= L_MIN) & (l <= L_MAX), ok, 0.0)

    def head(h, zero, history, ok):
        always = lax.broadcasted_iota(jnp.int32, (8, 128), 0) >= zero
        acc = None
        for t0 in range(0, STEPS, ST):
            kblk, qb, u0 = _step(t0)

            def put(r, lanes, a, b):
                pm[(t0 - u0 + r // CK) % PM][r % CK // 2:r % CK // 2 + 8, lanes] = _pack(a, b)

            lo, hi = (MXU_KEYS * u // NT // 16 * 16 for u in (u0, u0 + ST))
            s = _mm(pltpu.bitcast(k_s[h, kblk, lo // 2:hi // 2, :], BF16), query_weights(h, qb))
            e = jnp.exp2(s)
            for r in range(0, hi - lo, 16):
                for t in range(NT):
                    put(lo + r, _tile(t), e[r:r + 8, _tile(t)], e[r + 8:r + 16, _tile(t)])
            if t0 >= LAG:
                acc, parts = accumulate(t0 - LAG, h, h + 1, zero, acc)
            else:
                acc, parts = accumulate(STEPS - LAG + t0, jnp.maximum(h - 1, 0), h, zero, acc)

            history.append([s[r:r + 8, 0:128] for r in range(0, hi - lo, 8)]
                           + [part[r:r + 8, 0:128] for part in parts for r in range(0, VM, 8)])
            kb, kb_next = (kb0, kb1) if kblk % 2 == 0 else (kb1, kb0)
            for u in range(u0, u0 + ST):
                q = [jnp.broadcast_to(qf_s[h, qb, d:d + 1, _tile(u)], (8, 128)) for d in range(DH)]
                for d in range(DH):
                    when = (u - u0 - 0.66 + d / DH) / ST
                    back = -math.floor(when)
                    if back < len(history):
                        results = history[-1 - back]
                        q[d] = jnp.where(always, q[d], results[int(len(results) * (when + back))])
                scores = [None] * G
                for g0 in range(0, G, 2):
                    for d in range(DH):
                        for g in (g0, g0 + 1):
                            term = kb[(g * DH + d) * 8:(g * DH + d + 1) * 8, :] * q[d]
                            scores[g] = term if d == 0 else scores[g] + term
                for g in range(0, G, 2):
                    put(MXU_KEYS + 8 * g, _tile(u), jnp.exp2(scores[g]), jnp.exp2(scores[g + 1]))
                i, n, nxt = qb * NT + u, NB * NT, (kblk + 1) % NB
                h_nxt = h if nxt else jnp.minimum(h + 1, H - 1)
                spread_keys(kb_next, lambda r, d: kf_s[h_nxt, nxt, r, d], range(G * DH * i // n, G * DH * (i + 1) // n))
                if i == n - 2:
                    ok = check(h, kblk, ok)
        return ok

    def two_heads(i, carry):
        history, ok = [], ok_s[0]
        for h in (2 * i, 2 * i + 1):
            zero = lax.shift_right_logical(h, 10)
            ok = head(h, zero, history, ok)
        ok_s[0] = ok
        return carry + zero

    zero = lax.fori_loop(0, H // 2, two_heads, 0)
    acc, ok = None, ok_s[0]
    for t0 in range(STEPS - LAG, STEPS, ST):
        acc, _ = accumulate(t0, H - 1, H, 0, acc)
    for qb in range(NB):
        ok = check(H, qb, ok)

    @pl.when(jnp.min(ok) < 0.5)
    def _():
        def shifted_softmax(i, carry):
            h, qb = i // NB, i % NB
            w = query_weights(h, qb)

            def scores(t):
                return _mm(pltpu.bitcast(k_s[h, t // NT, _ds(t % NT * (CK // 2), CK // 2, 8), :], BF16), w)

            def row_max(t, m):
                return jnp.maximum(m, jnp.max(scores(t), axis=0, keepdims=True))

            m = lax.fori_loop(0, S // CK, row_max, jnp.full((1, BQ), -jnp.inf, F32))

            def weigh(t, o):
                return o + _mm(vt_s[h, t // NT, :, _ds(t % NT * CK, CK, CK)], jnp.exp2(scores(t) - m).astype(BF16))

            o_s[h + 1, qb] = lax.fori_loop(0, S // CK, weigh, jnp.zeros((VM, BQ), F32))
            return carry

        lax.fori_loop(0, H * NB, shifted_softmax, 0)

    wo_cp.wait()
    for cp in w_cp[3:]:
        cp.wait()
    b1, b2 = (jnp.concatenate([b[i:i + 1] for i in range(b.shape[0])], axis=1)
              for b in (b1_v[0].astype(F32), b2_v[0].astype(F32)))

    def rows(j):
        return _ds(j * TB, TB, TB)

    def attend(j):
        def head_rows(h):
            acc = o_s[h + 1, j // 2, :, _ds(j % 2 * TB, TB, TB)]
            inv = 1.0 / jnp.broadcast_to(acc[DH:DH + 1], (8, TB))
            return jnp.concatenate([acc[r:r + 8] * inv for r in range(0, VM, 8)], axis=0)[0:DH]

        att = jnp.concatenate([head_rows(h) for h in range(H)], axis=0).T
        res = x_v[rows(j), :].astype(F32) + jnp.concatenate(
            [_mm(att[r:r + HB].astype(BF16), wo_v[...]) for r in (0, HB)], axis=0)
        h_s[j % 4] = res
        hn = _layernorm(res)
        for i, term in enumerate(_lhs_terms(*_split(hn, HB, KS))):
            hn_s[i] = term.astype(BF16)
        hr_s[...] = hn[:, 2 * KS:].astype(BF16)

    def hidden_inputs():
        return [hn_s[i] for i in range(7)], hr_s[...]

    def hidden(terms, rest, jobs=()):
        if jobs:
            terms = [beside(term, zero, jobs[i::7]) for i, term in enumerate(terms)]
        extra = _split(_mm(rest, w1_v[2 * KS:, :]) + b1, HB, HF)
        quads = _quadrants(*_products((1, 3, 2, 4, 0, 5, 6), lambda i: terms[i], lambda i: pltpu.bitcast(w1_s[i], BF16)))
        return [jnp.square(jnp.maximum(q + e, 0.0)) for q, e in zip(quads, extra)]

    def store_hidden(a):
        for i, term in enumerate(_lhs_terms(*a) + (a[1], a[2])):
            a_s[i] = term.astype(BF16)

    def output_wide(j):
        y = _join(*_quadrants(*_products(range(7), lambda i: a_s[i], lambda i: pltpu.bitcast(w2_s[i], BF16))))
        out_v[rows(j), 0:2 * KS] = (h_s[j % 4, :, 0:2 * KS] + (y + b2[:, 0:2 * KS])).astype(BF16)
        return _join(a_s[2], a_s[7], a_s[8], a_s[3])

    def output_rest(j, a):
        y = _mm(a, w2_v[:, 2 * KS:]) + b2[:, 2 * KS:]
        out_v[rows(j), 2 * KS:] = (h_s[j % 4, :, 2 * KS:] + y).astype(BF16)

    def out_copy(i, r):
        return pltpu.make_async_copy(out_v.at[r, :], out_hbm.at[0, r, :], out_sem.at[i])

    def feed_forward(j, carry):
        inputs = hidden_inputs()
        a = output_wide(j)
        attend(j + 2)
        store_hidden(hidden(*inputs))
        output_rest(j, a)
        out_copy(j, rows(j)).start()
        return carry

    n = S // TB
    attend(0)
    inputs = hidden_inputs()
    attend(1)
    store_hidden(hidden(*inputs, [(w2_s, w2_v, HF, KS, r) for r in range(0, HF, 16)]))
    lax.fori_loop(0, n - 2, feed_forward, 0)
    a_last = hidden(*hidden_inputs())
    output_rest(n - 2, output_wide(n - 2))
    out_copy(n - 2, rows(n - 2)).start()
    a_last = _join(*a_last).astype(BF16)
    cuts = (0, HB, HB + HB // 2, TB)
    pieces = [pl.ds(S - TB + lo, hi - lo) for lo, hi in zip(cuts, cuts[1:])]
    for i, (lo, hi) in enumerate(zip(cuts, cuts[1:])):
        y = h_s[(n - 1) % 4, lo:hi, :] + (_mm(a_last[lo:hi], w2_v[...]) + b2)
        out_v[pieces[i], :] = y.astype(BF16)
        out_copy(n - 1 + i, pieces[i]).start()
    for i, r in enumerate([rows(j) for j in range(n - 1)] + pieces):
        out_copy(i, r).wait()


@jax.jit
def pallas_sequential_preLN__softmax_full_mha__dense_activation_squared_relu__prompt_kernel(
    A_x: jax.Array,
    A_wqkv: jax.Array,
    A_wo: jax.Array,
    B_x: jax.Array,
    B_w1: jax.Array,
    B_b1: jax.Array,
    B_w2: jax.Array,
    B_b2: jax.Array,
):
    del B_x
    hbm = pl.BlockSpec(memory_space=pl.ANY)
    scratch = [
        pltpu.VMEM((S, D), BF16),
        pltpu.VMEM((D, D), BF16),
        pltpu.VMEM((D, D), BF16),
        pltpu.VMEM((D, D), BF16),
        pltpu.VMEM((D, D), BF16),
        pltpu.VMEM((D, F), BF16),
        pltpu.VMEM((F, D), BF16),
        pltpu.VMEM((7, F // 128, 128), BF16),
        pltpu.VMEM((2, D // 128, 128), BF16),
        pltpu.VMEM((NB, BQ, D), BF16),
        pltpu.VMEM((NB, BQ // 2, D), U32),
        pltpu.VMEM((H, NB, BQ // 2, 128), U32),
        pltpu.VMEM((H, NB, 8 * G, DH), F32),
        pltpu.VMEM((H, NB, 16, BQ), U32),
        pltpu.VMEM((H, NB, VM, BQ), F32),
        pltpu.VMEM((H, NB, VM, BQ), F32),
        pltpu.VMEM((H + 1, NB, VM, BQ), F32),
        pltpu.VMEM((G * DH * 8, 128), F32),
        pltpu.VMEM((G * DH * 8, 128), F32),
        pltpu.VMEM((2, 8, BQ), F32),
        pltpu.VMEM((S, D), BF16),
        pltpu.VMEM((4, TB, D), F32),
        pltpu.VMEM((7, HB, KS), BF16),
        pltpu.VMEM((TB, D - 2 * KS), BF16),
        pltpu.VMEM((9, HB, HF), BF16),
        pltpu.VMEM((7, KS // 2, HF), U32),
        pltpu.VMEM((7, HF // 2, KS), U32),
        pltpu.SemaphoreType.DMA((NB + 8,)),
        pltpu.SemaphoreType.DMA((S // TB + 2,)),
    ]
    scratch += [pltpu.VMEM((CK // 2, BQ), U32)] * PM
    return pl.pallas_call(
        _kernel,
        out_shape=jax.ShapeDtypeStruct((1, S, D), BF16),
        in_specs=[hbm] * 7,
        out_specs=hbm,
        scratch_shapes=scratch,
        compiler_params=pltpu.CompilerParams(vmem_limit_bytes=100 * 2**20),
    )(A_x, A_wqkv, A_wo, B_w1, B_b1.reshape(F // 128, 128), B_w2, B_b2.reshape(D // 128, 128))
```

```python
import math

import jax
import jax.numpy as jnp
from jax import lax
import jax.experimental.pallas as pl
import jax.experimental.pallas.tpu as pltpu

S, D, F, H = 2048, 640, 1536, 32
DH = D // H
VM = 24
BQ = 512
NT = BQ // 128
NB = S // BQ
CK = 128
G = 10
MXU_KEYS = BQ - 8 * G
ST = 2
LAG = NT
PM = 2 * NT
STEPS = NB * NB * NT
TB = 256
HB, KS, HF = TB // 2, 256, F // 2
RB = 64
X0 = 320
EPS = 1e-5
Q_SCALE = DH ** -0.5 * math.log2(math.e)
L_MIN, L_MAX, V_MAX = 2.0 ** -60, 2.0 ** 100, 2.0 ** 20
F32, BF16, U32 = jnp.float32, jnp.bfloat16, jnp.uint32


def _layernorm(x):
    xc = x - jnp.mean(x, axis=-1, keepdims=True)
    return xc * lax.rsqrt(jnp.mean(xc * xc, axis=-1, keepdims=True) + EPS)


def _mm(a, b):
    return jnp.dot(a, b, preferred_element_type=F32)


def _tile(t):
    return slice(t * 128, (t + 1) * 128)


def _ds(start, size, align):
    return pl.ds(start if isinstance(start, int) else pl.multiple_of(start, align), size)


def _pack(a, b):
    return jnp.concatenate(
        [pltpu.bitcast(jnp.concatenate([a[:, _tile(t)], b[:, _tile(t)]], axis=0).astype(BF16), U32)
         for t in range(a.shape[1] // 128)], axis=1)


def _lhs_terms(a11, a12, a21, a22):
    return a11 + a22, a21 + a22, a11, a22, a11 + a12, a21 - a11, a12 - a22


def _rhs_terms(b11, b12, b21, b22):
    return b11 + b22, b11, b12 - b22, b21 - b11, b22, b11 + b12, b21 + b22


def _quadrants(m1, m2, m3, m4, m5, m6, m7):
    return m1 + m4 - m5 + m7, m3 + m5, m2 + m4, m1 - m2 + m3 + m6


def _products(order, lhs, rhs):
    m = {i: _mm(lhs(i), rhs(i)) for i in order}
    return [m[i] for i in range(7)]


def _split(a, r, c):
    return a[:r, :c], a[:r, c:2 * c], a[r:2 * r, :c], a[r:2 * r, c:2 * c]


def _join(c11, c12, c21, c22):
    return jnp.concatenate([jnp.concatenate([c11, c12], axis=1), jnp.concatenate([c21, c22], axis=1)], axis=0)


def _step(t):
    return t // (NB * NT), t // NT % NB, t % NT


def _kernel(x_hbm, wqkv_hbm, wo_hbm, w1_hbm, b1_hbm, w2_hbm, b2_hbm, out_hbm,
            x_v, wq_v, wk_v, wv_v, wo_v, w1_v, w2_v, b1_v, b2_v,
            xn_s, kraw_s, k_s, kf_s, qw_s, qf_s, vt_s, o_s, kb0, kb1, ok_s, out_v,
            h_s, hn_s, hr_s, a_s, w1_s, w2_s, att_s, in_sem, out_sem, *pm):
    def x_copy(half, part):
        r = _ds(half * (S // 2) + part * X0, S // 2 - X0 if part else X0, RB)
        return pltpu.make_async_copy(x_hbm.at[0, r, :], x_v.at[r, :], in_sem.at[2 * half + part])

    x_cp = [x_copy(half, part) for half in range(2) for part in range(2)]
    wk_cp, wo_cp, *w_cp = [pltpu.make_async_copy(src, dst, in_sem.at[NB + i]) for i, (src, dst) in enumerate((
        (wqkv_hbm.at[:, pl.ds(D, D)], wk_v), (wo_hbm, wo_v),
        (wqkv_hbm.at[:, pl.ds(2 * D, D)], wv_v), (wqkv_hbm.at[:, pl.ds(0, D)], wq_v),
        (w1_hbm, w1_v), (w2_hbm, w2_v), (b1_hbm, b1_v.at[0]), (b2_hbm, b2_v.at[0])))]

    for cp in [x_cp[0], wk_cp] + x_cp[1:] + w_cp[:3]:
        cp.start()
    ok_s[0] = jnp.ones((8, BQ), F32)
    for t in range(STEPS - LAG, STEPS):
        pm[t % PM][...] = jnp.zeros((CK // 2, BQ), U32)
    o_s[0] = jnp.ones((NB, VM, BQ), F32)
    x_cp[0].wait()
    xn_s[0, 0:RB, :] = _layernorm(x_v[0:RB, :].astype(F32)).astype(BF16)
    wk_cp.wait()

    def window(h):
        return h * DH // 16 * 16

    def project_keys(half, carry):
        def normed(r):
            c, o = 2 * half + r // BQ, r % BQ
            xn = _layernorm(x_v[_ds(c * BQ + o, RB, RB), :].astype(F32)).astype(BF16)
            xn_s[c, o:o + RB, :] = xn
            return xn

        @pl.when(half == 1)
        def _():
            x_cp[2].wait()
            normed(0)

        xn = xn_s[2 * half, 0:RB, :]
        for r0 in range(0, 2 * BQ, RB):
            if r0 + RB == X0:
                x_copy(half, 1).wait()
            k = _mm(xn, wk_v[...])
            if r0 + RB < 2 * BQ:
                xn = normed(r0 + RB)
            c, o = 2 * half + r0 // BQ, r0 % BQ
            for r in range(0, RB, 16):
                kraw_s[c, (o + r) // 2:(o + r) // 2 + 8, :] = _pack(k[r:r + 8], k[r + 8:r + 16])
        return carry

    def store_keys(c):
        k = kraw_s[c]
        k_vpu = pltpu.bitcast(k[MXU_KEYS // 2:], BF16).astype(F32)
        for h in range(H):
            t, off = divmod(window(h), 128)
            win = k[:, _tile(t)]
            if off:
                win = pltpu.roll(win, 128 - off, axis=1)
            if off + 32 > 128:
                lane = lax.broadcasted_iota(jnp.int32, win.shape, 1)
                win = jnp.where(lane < 128 - off, win, pltpu.roll(k[:, _tile(t + 1)], 128 - off, axis=1))
            k_s[h, c] = win
            kf_s[h, c] = k_vpu[:, h * DH:(h + 1) * DH]

    def store_queries(c, q):
        q = (q * Q_SCALE).astype(BF16).astype(F32).T
        row = lax.broadcasted_iota(jnp.int32, (8, BQ), 0)
        for h in range(H):
            w = []
            for r in range(window(h), window(h) + 32, 8):
                lo, hi = h * DH - r, (h + 1) * DH - r
                if lo >= 8 or hi <= 0:
                    w.append(jnp.zeros((8, BQ), F32))
                elif lo > 0 or hi < 8:
                    w.append(jnp.where((row >= lo) & (row < hi), q[r:r + 8], 0.0))
                else:
                    w.append(q[r:r + 8])
            qw_s[h, c, 0:8, :] = _pack(w[0], w[1])
            qw_s[h, c, 8:16, :] = _pack(w[2], w[3])
            qf_s[h, c, 0:DH, :] = q[h * DH:(h + 1) * DH]

    def store_values(c, v):
        v = v.astype(BF16).astype(F32).T
        small = jnp.where(jnp.abs(v) <= V_MAX, 1.0, 0.0)
        ok_s[0] = jnp.minimum(ok_s[0], jnp.min(small.reshape(D // 8, 8, BQ), axis=0))
        for h in range(H):
            vt_s[h, c, 0:DH, :] = v[h * DH:(h + 1) * DH]
            vt_s[h, c, DH:VM, :] = jnp.ones((VM - DH, BQ), F32)

    def spread_keys(kb, k, items):
        for i in items:
            d, g = divmod(i, G)
            kb[(g * DH + d) * 8:(g * DH + d + 1) * 8, :] = jnp.broadcast_to(k(slice(8 * g, 8 * g + 8), slice(d, d + 1)), (8, 128))

    def strassen_weights(ref, w_v, rows, cols, r):
        top = w_v[_ds(r, 16, 16), 0:2 * cols].astype(F32)
        bot = w_v[_ds(rows + r, 16, 16), 0:2 * cols].astype(F32)
        token = None
        for i, term in enumerate(_rhs_terms(top[:, :cols], top[:, cols:], bot[:, :cols], bot[:, cols:])):
            packed = _pack(term[0:8], term[8:16])
            ref[i, _ds(r // 2, 8, 8), :] = packed
            for t in range(cols // 128):
                token = packed[:, _tile(t)] if token is None else token | packed[:, _tile(t)]
        return token

    def beside(lhs, zero, jobs):
        token = None
        for job in jobs:
            t = strassen_weights(*job)
            token = t if token is None else token | t
        always = lax.broadcasted_iota(jnp.int32, (16, 128), 0) >= zero
        corner = jnp.where(always, lhs[0:16, 0:128], pltpu.bitcast(token, BF16))
        return jnp.concatenate([jnp.concatenate([corner, lhs[0:16, 128:]], axis=1), lhs[16:]], axis=0)

    def project_queries_values(half, carry):
        zero = lax.shift_right_logical(half, 10)
        jobs = [(w1_s, w1_v, KS, HF, half * (KS // 2) + r) for r in range(0, KS // 2, 16)]
        for i in range(2):
            c = 2 * half + i
            q = _mm(xn_s[c], wq_v[...])
            store_keys(c)
            if i == 0:
                k0 = pltpu.bitcast(kraw_s[0, MXU_KEYS // 2:, 0:128], BF16).astype(F32)
                spread_keys(kb0, lambda r, d: k0[r, d], range(G * DH))
            v = jnp.concatenate([_mm(beside(xn_s[c, r:r + 128, :], zero, [jobs.pop()]), wv_v[...])
                                 for r in range(0, BQ, 128)], axis=0)
            store_queries(c, q)
            store_values(c, v)
        return carry

    lax.fori_loop(0, 2, project_keys, 0)
    for cp in w_cp[:3]:
        cp.wait()
    lax.fori_loop(0, 2, project_queries_values, 0)
    for cp in [wo_cp] + w_cp[3:]:
        cp.start()

    def query_weights(h, qb):
        return jnp.concatenate([pltpu.bitcast(qw_s[h, qb], BF16), jnp.zeros((96, BQ), BF16)], axis=0)

    def accumulate(t0, h, slot, zero, acc):
        parts = []
        for t in range(t0, t0 + ST):
            kblk, qb, u = _step(t)
            p = pltpu.bitcast(pm[t % PM][_ds(zero * 8, CK // 2, 8), :], BF16)
            parts.append(_mm(vt_s[h, kblk, :, _tile(u)], p))
            acc = parts[-1] if u == 0 else acc + parts[-1]
            if u == NT - 1:
                o_s[slot, qb] = acc + o_s[slot, qb] if kblk else acc
        return acc, parts

    def check(slot, qb, ok):
        l = jnp.broadcast_to(o_s[slot, qb, DH:DH + 1, :], (8, BQ))
        return jnp.where((l >= L_MIN) & (l <= L_MAX), ok, 0.0)

    def head(h, zero, history, ok):
        always = lax.broadcasted_iota(jnp.int32, (8, 128), 0) >= zero
        acc = None
        for t0 in range(0, STEPS, ST):
            kblk, qb, u0 = _step(t0)

            def put(r, lanes, a, b):
                pm[(t0 - u0 + r // CK) % PM][r % CK // 2:r % CK // 2 + 8, lanes] = _pack(a, b)

            lo, hi = (MXU_KEYS * u // NT // 16 * 16 for u in (u0, u0 + ST))
            s = _mm(pltpu.bitcast(k_s[h, kblk, lo // 2:hi // 2, :], BF16), query_weights(h, qb))
            e = jnp.exp2(s)
            for r in range(0, hi - lo, 16):
                for t in range(NT):
                    put(lo + r, _tile(t), e[r:r + 8, _tile(t)], e[r + 8:r + 16, _tile(t)])
            if t0 >= LAG:
                acc, parts = accumulate(t0 - LAG, h, h + 1, zero, acc)
            else:
                acc, parts = accumulate(STEPS - LAG + t0, jnp.maximum(h - 1, 0), h, zero, acc)

            history.append([s[r:r + 8, 0:128] for r in range(0, hi - lo, 8)]
                           + [part[r:r + 8, 0:128] for part in parts for r in range(0, VM, 8)])
            kb, kb_next = (kb0, kb1) if kblk % 2 == 0 else (kb1, kb0)
            for u in range(u0, u0 + ST):
                q = [jnp.broadcast_to(qf_s[h, qb, d:d + 1, _tile(u)], (8, 128)) for d in range(DH)]
                for d in range(DH):
                    when = (u - u0 - 0.66 + d / DH) / ST
                    back = -math.floor(when)
                    if back < len(history):
                        results = history[-1 - back]
                        q[d] = jnp.where(always, q[d], results[int(len(results) * (when + back))])
                scores = [None] * G
                for g0 in range(0, G, 2):
                    for d in range(DH):
                        for g in (g0, g0 + 1):
                            term = kb[(g * DH + d) * 8:(g * DH + d + 1) * 8, :] * q[d]
                            scores[g] = term if d == 0 else scores[g] + term
                for g in range(0, G, 2):
                    put(MXU_KEYS + 8 * g, _tile(u), jnp.exp2(scores[g]), jnp.exp2(scores[g + 1]))
                i, n, nxt = qb * NT + u, NB * NT, (kblk + 1) % NB
                h_nxt = h if nxt else jnp.minimum(h + 1, H - 1)
                spread_keys(kb_next, lambda r, d: kf_s[h_nxt, nxt, r, d], range(G * DH * i // n, G * DH * (i + 1) // n))
                if i == n - 2:
                    ok = check(h, kblk, ok)
        return ok

    def two_heads(i, carry):
        history, ok = [], ok_s[0]
        for h in (2 * i, 2 * i + 1):
            zero = lax.shift_right_logical(h, 10)
            ok = head(h, zero, history, ok)
        ok_s[0] = ok
        return carry + zero

    zero = lax.fori_loop(0, H // 2, two_heads, 0)
    acc, ok = None, ok_s[0]
    for t0 in range(STEPS - LAG, STEPS, ST):
        acc, _ = accumulate(t0, H - 1, H, 0, acc)
    for qb in range(NB):
        ok = check(H, qb, ok)

    def gather_heads(j):
        def head_rows(h):
            acc = o_s[h + 1, j // 2, :, _ds(j % 2 * TB, TB, TB)]
            inv = 1.0 / jnp.broadcast_to(acc[DH:DH + 1], (8, TB))
            return jnp.concatenate([acc[r:r + 8] * inv for r in range(0, VM, 8)], axis=0)[0:DH]

        return jnp.concatenate([head_rows(h) for h in range(H)], axis=0).T.astype(BF16)

    att_s[...] = gather_heads(0)

    @pl.when(jnp.min(ok) < 0.5)
    def _():
        def shifted_softmax(i, carry):
            h, qb = i // NB, i % NB
            w = query_weights(h, qb)

            def scores(t):
                return _mm(pltpu.bitcast(k_s[h, t // NT, _ds(t % NT * (CK // 2), CK // 2, 8), :], BF16), w)

            def row_max(t, m):
                return jnp.maximum(m, jnp.max(scores(t), axis=0, keepdims=True))

            m = lax.fori_loop(0, S // CK, row_max, jnp.full((1, BQ), -jnp.inf, F32))

            def weigh(t, o):
                return o + _mm(vt_s[h, t // NT, :, _ds(t % NT * CK, CK, CK)], jnp.exp2(scores(t) - m).astype(BF16))

            o_s[h + 1, qb] = lax.fori_loop(0, S // CK, weigh, jnp.zeros((VM, BQ), F32))
            return carry

        lax.fori_loop(0, H * NB, shifted_softmax, 0)
        att_s[...] = gather_heads(0)

    wo_cp.wait()
    for cp in w_cp[3:]:
        cp.wait()
    b1, b2 = (jnp.concatenate([b[i:i + 1] for i in range(b.shape[0])], axis=1)
              for b in (b1_v[0].astype(F32), b2_v[0].astype(F32)))

    def rows(j):
        return _ds(j * TB, TB, TB)

    def attend(j, att):
        res = x_v[rows(j), :].astype(F32) + jnp.concatenate(
            [_mm(att[r:r + HB], wo_v[...]) for r in (0, HB)], axis=0)
        h_s[j % 4] = res
        hn = _layernorm(res)
        for i, term in enumerate(_lhs_terms(*_split(hn, HB, KS))):
            hn_s[i] = term.astype(BF16)
        hr_s[...] = hn[:, 2 * KS:].astype(BF16)

    def hidden_inputs():
        return [hn_s[i] for i in range(7)], hr_s[...]

    def hidden(terms, rest, jobs=()):
        if jobs:
            terms = [beside(term, zero, jobs[i::7]) for i, term in enumerate(terms)]
        extra = _split(_mm(rest, w1_v[2 * KS:, :]) + b1, HB, HF)
        quads = _quadrants(*_products((1, 3, 2, 4, 0, 5, 6), lambda i: terms[i], lambda i: pltpu.bitcast(w1_s[i], BF16)))
        return [jnp.square(jnp.maximum(q + e, 0.0)) for q, e in zip(quads, extra)]

    def store_hidden(a):
        for i, term in enumerate(_lhs_terms(*a) + (a[1], a[2])):
            a_s[i] = term.astype(BF16)

    def output_wide(j):
        y = _join(*_quadrants(*_products(range(7), lambda i: a_s[i], lambda i: pltpu.bitcast(w2_s[i], BF16))))
        out_v[rows(j), 0:2 * KS] = (h_s[j % 4, :, 0:2 * KS] + (y + b2[:, 0:2 * KS])).astype(BF16)
        return _join(a_s[2], a_s[7], a_s[8], a_s[3])

    def output_rest(j, a):
        y = _mm(a, w2_v[:, 2 * KS:]) + b2[:, 2 * KS:]
        out_v[rows(j), 2 * KS:] = (h_s[j % 4, :, 2 * KS:] + y).astype(BF16)

    def out_copy(i, r):
        return pltpu.make_async_copy(out_v.at[r, :], out_hbm.at[0, r, :], out_sem.at[i])

    def feed_forward(j, carry):
        inputs = hidden_inputs()
        a = output_wide(j)
        attend(j + 2, gather_heads(j + 2))
        store_hidden(hidden(*inputs))
        output_rest(j, a)
        out_copy(j, rows(j)).start()
        return carry

    n = S // TB
    attend(0, att_s[...])
    inputs = hidden_inputs()
    attend(1, gather_heads(1))
    store_hidden(hidden(*inputs, [(w2_s, w2_v, HF, KS, r) for r in range(0, HF, 16)]))
    lax.fori_loop(0, n - 2, feed_forward, 0)
    a_last = hidden(*hidden_inputs())
    output_rest(n - 2, output_wide(n - 2))
    out_copy(n - 2, rows(n - 2)).start()
    a_last = _join(*a_last).astype(BF16)
    cuts = (0, HB, HB + HB // 2, TB)
    pieces = [pl.ds(S - TB + lo, hi - lo) for lo, hi in zip(cuts, cuts[1:])]
    for i, (lo, hi) in enumerate(zip(cuts, cuts[1:])):
        y = h_s[(n - 1) % 4, lo:hi, :] + (_mm(a_last[lo:hi], w2_v[...]) + b2)
        out_v[pieces[i], :] = y.astype(BF16)
        out_copy(n - 1 + i, pieces[i]).start()
    for i, r in enumerate([rows(j) for j in range(n - 1)] + pieces):
        out_copy(i, r).wait()


@jax.jit
def pallas_sequential_preLN__softmax_full_mha__dense_activation_squared_relu__prompt_kernel(
    A_x: jax.Array,
    A_wqkv: jax.Array,
    A_wo: jax.Array,
    B_x: jax.Array,
    B_w1: jax.Array,
    B_b1: jax.Array,
    B_w2: jax.Array,
    B_b2: jax.Array,
):
    del B_x
    hbm = pl.BlockSpec(memory_space=pl.ANY)
    scratch = [
        pltpu.VMEM((S, D), BF16),
        pltpu.VMEM((D, D), BF16),
        pltpu.VMEM((D, D), BF16),
        pltpu.VMEM((D, D), BF16),
        pltpu.VMEM((D, D), BF16),
        pltpu.VMEM((D, F), BF16),
        pltpu.VMEM((F, D), BF16),
        pltpu.VMEM((7, F // 128, 128), BF16),
        pltpu.VMEM((2, D // 128, 128), BF16),
        pltpu.VMEM((NB, BQ, D), BF16),
        pltpu.VMEM((NB, BQ // 2, D), U32),
        pltpu.VMEM((H, NB, BQ // 2, 128), U32),
        pltpu.VMEM((H, NB, 8 * G, DH), F32),
        pltpu.VMEM((H, NB, 16, BQ), U32),
        pltpu.VMEM((H, NB, VM, BQ), F32),
        pltpu.VMEM((H, NB, VM, BQ), F32),
        pltpu.VMEM((H + 1, NB, VM, BQ), F32),
        pltpu.VMEM((G * DH * 8, 128), F32),
        pltpu.VMEM((G * DH * 8, 128), F32),
        pltpu.VMEM((2, 8, BQ), F32),
        pltpu.VMEM((S, D), BF16),
        pltpu.VMEM((4, TB, D), F32),
        pltpu.VMEM((7, HB, KS), BF16),
        pltpu.VMEM((TB, D - 2 * KS), BF16),
        pltpu.VMEM((9, HB, HF), BF16),
        pltpu.VMEM((7, KS // 2, HF), U32),
        pltpu.VMEM((7, HF // 2, KS), U32),
        pltpu.VMEM((TB, D), BF16),
        pltpu.SemaphoreType.DMA((NB + 8,)),
        pltpu.SemaphoreType.DMA((S // TB + 2,)),
    ]
    scratch += [pltpu.VMEM((CK // 2, BQ), U32)] * PM
    return pl.pallas_call(
        _kernel,
        out_shape=jax.ShapeDtypeStruct((1, S, D), BF16),
        in_specs=[hbm] * 7,
        out_specs=hbm,
        scratch_shapes=scratch,
        compiler_params=pltpu.CompilerParams(vmem_limit_bytes=100 * 2**20),
    )(A_x, A_wqkv, A_wo, B_w1, B_b1.reshape(F // 128, 128), B_w2, B_b2.reshape(D // 128, 128))
```
